```python
import os as _os
_os.environ.setdefault("JAX_PLATFORMS", "cpu")
import jax
import jax.numpy as jnp

def _softmax(x, axis=-1):
    return jax.nn.softmax(x, axis=axis)
def _gelu(x):
    return jax.nn.gelu(x, approximate=True)
def _silu(x):
    return jax.nn.silu(x)
def _sigmoid(x):
    return jax.nn.sigmoid(x)
def _layernorm(x, axis=-1, eps=1e-5):
    m = jnp.mean(x, axis=axis, keepdims=True)
    v = jnp.var(x, axis=axis, keepdims=True)
    return (x - m) / jnp.sqrt(v + eps)
def _scatter_add(tgt, idx, src, axis=0):
    return tgt.at[idx].add(src)
def _segment_sum(src, seg, n):
    return jax.ops.segment_sum(src, seg, n)
class _Rng:
    def __init__(self, key):
        self._k = key
    def _next(self):
        self._k, sub = jax.random.split(self._k)
        return sub
    def normal(self, shape):
        return jax.random.normal(self._next(), shape, dtype=jnp.bfloat16)
    def randint(self, lo, hi, shape):
        return jax.random.randint(self._next(), shape, lo, hi, dtype=jnp.int32)
    def uniform(self, shape, lo=0.0, hi=1.0):
        return jax.random.uniform(self._next(), shape, jnp.bfloat16, lo, hi)
    def permutation(self, n):
        return jax.random.permutation(self._next(), n)


kernel_name = 'gated_mix__ssm_conv_h3__mixer_s_mlp__prompt'

def setup_inputs():
    _rng = _Rng(jax.random.key(int.from_bytes(__import__("os").urandom(4), "little")))
    _w = (lambda a: (lambda t: t.astype(jnp.bfloat16) if jnp.issubdtype(t.dtype, jnp.floating) else t)(jnp.asarray(a)))
    def _A_setup():
        B, S, D = 1, 2048, 576
        ks = 4
        return {
            "q": _w((lambda *s: _rng.normal(s) * 0.05)(B, S, D)),
            "k": _w((lambda *s: _rng.normal(s) * 0.4)(B, S, D)),
            "v": _w((lambda *s: _rng.normal(s) * 0.4)(B, S, D)),
            "shift_k": _w((lambda *s: _rng.normal(s) * 0.4)(D, ks) * 0.5),
            "ssm_k": _w((lambda *s: _rng.normal(s) * 0.4)(D, S) * (1.0 / S ** 0.5)),
            "ssm_D": _w((lambda *s: _rng.normal(s) * 0.4)(D)),
        }
    _A_in = _A_setup()

    def _B_setup():
        B, S, D, F = 1, 2048, 576, 4608
        return {
            "x":  _w((lambda *s: _rng.normal(s) * 0.05)(B, S, D)),
            "w1": _w((lambda *s: _rng.normal(s) * 0.2)(D, D) * (D ** -0.5)),
            "w2": _w((lambda *s: _rng.normal(s) * 0.2)(D, D) * (D ** -0.5)),
            "w3": _w((lambda *s: _rng.normal(s) * 0.2)(D, F) * (D ** -0.5)),
            "w4": _w((lambda *s: _rng.normal(s) * 0.2)(F, D) * (F ** -0.5)),
        }
    _B_in = _B_setup()

    return {
        "A_q": _A_in["q"],
        "A_k": _A_in["k"],
        "A_v": _A_in["v"],
        "A_shift_k": _A_in["shift_k"],
        "A_ssm_k": _A_in["ssm_k"],
        "A_ssm_D": _A_in["ssm_D"],
        "B_x": _B_in["x"],
        "B_w1": _B_in["w1"],
        "B_w2": _B_in["w2"],
        "B_w3": _B_in["w3"],
        "B_w4": _B_in["w4"],
        "gate_w": _w((lambda *s: _rng.normal(s) * 0.05)(576) * 16.0),
    }

def reference(A_q, A_k, A_v, A_shift_k, A_ssm_k, A_ssm_D, B_x, B_w1, B_w2, B_w3, B_w4, gate_w):
    def _A_ref(q, k, v, shift_k, ssm_k, ssm_D):
        B, S, D = q.shape
        ks = shift_k.shape[-1]
        k_pad = jnp.pad(k, ((0, 0), (ks - 1, 0), (0, 0)))
        k_shift = jnp.zeros_like(k)
        for t in range(ks):
            k_shift = k_shift + k_pad[:, t:t + S, :] * shift_k[:, ks - 1 - t][None, None, :]
        kv = k_shift * v
        L = 2 * S
        kv_pad = jnp.pad(kv, ((0, 0), (0, S), (0, 0)))
        kf_pad = jnp.pad(ssm_k, ((0, 0), (0, S)))
        kv_f = (lambda x, axes=(-2,-1): jnp.fft.rfft2(x.astype(jnp.float32), axes=axes))(kv_pad[:, None, :, :], axes=(1, 2))
        kf_f = (lambda x, axes=(-2,-1): jnp.fft.rfft2(x.astype(jnp.float32), axes=axes))(kf_pad[:, None, :], axes=(1, 2))
        kf_f = (lambda x, *d: x.transpose(*d))(kf_f, 1, 2, 0)
        y_f = kv_f * kf_f[None, :, :, :]
        y = (lambda x, s, axes=(-2,-1): jnp.fft.irfft2(x, s=s, axes=axes).astype(jnp.bfloat16))(y_f, (1, L), axes=(1, 2))[:, 0, :S, :]
        y = y + kv * ssm_D[None, None, :]
        return q * y

    def _B_ref(x, w1, w2, w3, w4):
        B, S, D = x.shape
        h = _gelu(_layernorm(x, axis=-1) @ w1)
        c = D // 4
        g0 = jnp.pad(h[:, :, 0*c:1*c], ((0, 0), (1, 0), (0, 0)))[:, :S, :]
        g1 = jnp.pad(h[:, :, 1*c:2*c], ((0, 0), (0, 1), (0, 0)))[:, 1:, :]
        g2 = jnp.pad(h[:, :, 2*c:3*c], ((0, 0), (2, 0), (0, 0)))[:, :S, :]
        g3 = jnp.pad(h[:, :, 3*c:   ], ((0, 0), (0, 2), (0, 0)))[:, 2:, :]
        hs = jnp.concatenate([g0, g1, g2, g3], axis=-1) @ w2
        x1 = x + hs
        h2 = _gelu(_layernorm(x1, axis=-1) @ w3) @ w4
        return x1 + h2

    x = A_q
    g = _sigmoid((x * gate_w).sum(-1, keepdims=True))
    a = _A_ref(x, A_k, A_v, A_shift_k, A_ssm_k, A_ssm_D)
    b = _B_ref(x, B_w1, B_w2, B_w3, B_w4)
    return g * a + (1 - g) * b
```

```python
import math

import jax
import jax.numpy as jnp
from jax import lax
from jax.experimental import pallas as pl
from jax.experimental.pallas import tpu as pltpu

bf16, f32, u32 = jnp.bfloat16, jnp.float32, jnp.uint32
S, D, F = 2048, 576, 4608
L = 128
NC = S // L
TF = 512
NF = F // TF
CG = D // NF
EPS = 1e-5
_C0 = math.sqrt(2.0 / math.pi)
GS = (_C0 * 0.044715) ** (1.0 / 3.0)
GA = _C0 / GS
NT = (((1,), (1,)), ((), ()))
QUADS = ((0, 0), (0, 1), (1, 0), (1, 1))
A_TERMS = (((1, 0, 0), (1, 1, 1)), ((1, 1, 0), (1, 1, 1)), ((1, 0, 0),), ((1, 1, 1),),
           ((1, 0, 0), (1, 0, 1)), ((1, 1, 0), (-1, 0, 0)), ((1, 0, 1), (-1, 1, 1)))
B_TERMS = (((1, 0, 0), (1, 1, 1)), ((1, 0, 0),), ((1, 0, 1), (-1, 1, 1)), ((1, 1, 0), (-1, 0, 0)),
           ((1, 1, 1),), ((1, 0, 0), (1, 0, 1)), ((1, 1, 0), (1, 1, 1)))
LONG = (0, 1, 2, 5)
QUARTER = (0, 192, 320, 448)
PAD = 8
SHIFTS = (1, -1, 2, -2)
cat = jnp.concatenate


def spec(shape, dtype):
    return jax.ShapeDtypeStruct(shape, dtype)


def gelu2(xs):
    return xs + xs * jnp.tanh(xs * (xs * xs + GA))


def dot(a, b):
    return jnp.dot(a, b, preferred_element_type=f32)


def dot_nt(a, b):
    return lax.dot_general(a, b, NT, preferred_element_type=f32)


def packed(x):
    return pltpu.bitcast(x.astype(bf16), u32)


def lin(terms, get):
    acc = None
    for sign, r, c in terms:
        v = get(r, c)
        if v is not None:
            acc = (v if sign > 0 else -v) if acc is None else (acc + v if sign > 0 else acc - v)
    return acc


def combine(get, ij):
    if ij == (0, 1):
        return get(2) + get(4)
    if ij == (1, 0):
        return get(1) + get(3)
    if ij == (0, 0):
        return (get(0) + get(6)) + (get(3) - get(4))
    return (get(0) + get(5)) + (get(2) - get(1))


def tree_sum(xs):
    while len(xs) > 1:
        xs = [xs[i] + xs[i + 1] if i + 1 < len(xs) else xs[i] for i in range(0, len(xs), 2)]
    return xs[0]


def merge(*lists):
    m = []
    for li, l in enumerate(lists):
        total, acc = sum(t[0] for t in l), 0
        for t in l:
            m.append(((acc + t[0] / 2) / total, li, t))
            acc += t[0]
    return [t for _, _, t in sorted(m, key=lambda e: e[:2])]


class Program:
    def __init__(self, lead, use, tune):
        self.lead, self.use, self.tune, self.pull = lead, use, tune[:5], tune[5:]
        self.steps, self.slots, self.outs = [], [], []
        self.load, self.prev = [0] * 4, [(0, 0)] * 4
        self.due, self.res = {}, {}

    def step(self, dots, fn, open_=True):
        k = len(self.steps)
        for j, (n, w, xp) in enumerate(dots):
            for m in range(w):
                u = min(range(4), key=lambda q: (self.load[q], q))
                t0, n0 = self.prev[u]
                units, plain, turned, end, every = self.tune
                if m == 0 and n0 and open_ and u < units:
                    off, rate = turned if xp else plain
                    self.slots += [(t0 + off * n0 / 8 + e * rate * n0 / 8, (k, j), 7 - e) for e in range(8 if xp else self.use)]
                self.outs += [(self.load[u] + e, k, j, e, m, u) for e in range(n)]
                self.prev[u] = (self.load[u], n)
                self.load[u] += n
        self.steps.append((len(dots), fn))

    def now(self):
        return sum(self.load) / 4

    def spread(self, tasks, t0, t1, first, limit):
        total, acc, last = sum(t[0] for t in tasks), 0, (first, 0)
        for n, (c, fn, *early) in enumerate(tasks):
            ts = t0 + (t1 - t0) * acc / total
            acc += c
            te = ts + self.tune[3] * (t1 - t0) * c / total
            t, last, vreg = min((s for s in self.slots if last <= s[1] < (limit, 0)), key=lambda s: (abs(s[0] - te), s[1]))
            self.due.setdefault(last, []).append((t, vreg, fn, ts - self.lead - sum(early) if n % self.tune[4] == 0 else -1,
                                                  n % self.pull[2] == 0))

    def gate(self, t, k, u=0):
        ready = [o for o in self.outs if o[0] <= t and o[1] < k and o[5] == u]
        if not ready:
            return None
        _, kk, j, e, m, _ = ready[-1]
        r = self.res[kk][j]
        m = min(m, r.shape[1] // L - 1)
        return r[16 * e:16 * e + 8, L * m:L * m + L]

    def emit(self):
        for k, (n, fn) in enumerate(self.steps):
            pull = lambda e: [g for g in (self.gate(e[0] - self.pull[0], k, u) for u in self.pull[1] * e[4]) if g is not None]
            due = [[(e[1], lambda e=e: list(e[2](self.gate(e[3], k))) + pull(e))
                    for e in sorted(self.due.get((k, j), []), key=lambda e: e[0])] for j in range(n)]
            self.res[k] = fn(due)


DEFAULT = dict(LEAD=20, LE=16, LX=14, UN=1, USE=6, PO=0, PR=1, TO=2, TR=0.5, EN=0.5, GE=1, PL=11, PU=(0, 1, 2, 3), XE=0, PE=2)


HEAD = dict(LE=6, UN=4, LX=10, EN=0, TO=2, LEAD=14, PU=(), XE=16, TR=0.75)
TAIL = dict(LEAD=18, TR=1, UN=4)


def build(H=HEAD, M=None, T=TAIL, RS=1, EA=8, EB=6, KW=50, CB=2, KG=2, KP=(4, 14, 24, 34), XP=(10, 20, 30, 40),
          IP=(100, 132, 164, 193), RG=112, LR=96, CK=(4, 14, 24, 34), CX=(10, 20, 30, 40), CI=(25, 45, 70, 95), TE=12,
          WP=(6, 6, 6, 6, 6), T7=20, XL=18, XW=7, FL=4, TS0=0.6, TS=0.3, L1=10):
    H, M, T = ({**DEFAULT, **(c or {})} for c in (H, M, T))
    long_ = [p1 in LONG and p2 in LONG for p1 in range(7) for p2 in range(7)]
    cols, nxt = [], 0
    for lg in long_:
        cols.append(nxt)
        nxt += 3 if lg else 2

    def kern(q_hbm, k_hbm, v_hbm, sh_hbm, kk_hbm, d_hbm, w1_hbm, w2_hbm, w3_hbm, w4_hbm, gw_hbm, o_hbm,
             q_v, kv_v, kk_v, w1_v, w2_v, w3_v, w4_v, sh_v, d_v, gw_v, o_v,
             pt_s, par_s, f_s, wt_s, st_s, r_s, xn_s, h_s, hs_s, x1_s, xq_s, xp_s, xa_s, g_s, ga_s,
             acc_s, p_s, u_s, b_s, a_s, c_s, kvp_s, y_s, z_s,
             sems):
        def cols_of(src, dst, a, b, sem):
            return pltpu.make_async_copy(src.at[:, pl.ds(a, b - a)], dst.at[:, pl.ds(a, b - a)], sem)

        def rows_of(src, dst, a, b, sem):
            return pltpu.make_async_copy(src.at[pl.ds(a, b - a), :], dst.at[pl.ds(a, b - a), pl.ds(0, S)], sem)

        def chunks(a, b, s):
            return [cols_of(w3_hbm, w3_v, TF * (a + 1), TF * min(b + 1, NF), s[0]),
                    cols_of(w4_hbm, w4_v, TF * a, TF * b, s[1]),
                    rows_of(k_hbm, kv_v.at[0], CG * a, CG * b, s[2]),
                    rows_of(v_hbm, kv_v.at[1], CG * a, CG * b, s[3]),
                    rows_of(kk_hbm, kk_v, CG * a, CG * b, s[4])]

        sem = [sems.at[j] for j in range(sems.shape[0])]
        small = [pltpu.make_async_copy(s, d, sem[j]) for j, (s, d) in enumerate(
            ((sh_hbm, sh_v), (d_hbm, d_v), (gw_hbm, gw_v)))]
        w1_copy = pltpu.make_async_copy(w1_hbm, w1_v, sem[3])
        q_first = cols_of(q_hbm, q_v.at[0], 0, 512, sem[4])
        q_second = [cols_of(q_hbm, q_v.at[0], a, a + 256, sem[3 + a // 256]) for a in (512, 768)]
        q_rest = [cols_of(q_hbm, q_v.at[0], 1024, S, sem[7]), pltpu.make_async_copy(w2_hbm, w2_v, sem[23])]
        early = [cols_of(w3_hbm, w3_v, 0, TF, sem[8])]
        then, late = chunks(0, 1, sem[13:18]), chunks(1, NF, sem[18:23])
        out = [[cols_of(o_v, o_hbm, 0, 1024, sem[24])]]
        out += [[cols_of(o_v, o_hbm, a, a + 256, sem[21 + a // 256]) for a in (c, c + 512)] for c in (1024, 1280)]

        for c in small + [w1_copy, q_first]:
            c.start()

        z_s[0] = 0
        n_i = lax.broadcasted_iota(jnp.int32, (L, L), 0)
        g_i = lax.broadcasted_iota(jnp.int32, (L, L), 1)
        ang = (((4 * g_i + 1) * n_i) & (4 * L - 1)).astype(f32) * (2.0 * math.pi / (4 * L))
        f_s[0, 0:64] = pltpu.bitcast(jnp.cos(ang).astype(bf16), u32)
        f_s[1, 0:64] = pltpu.bitcast(jnp.sin(ang).astype(bf16), u32)

        def stacked(ref, first, n):
            return cat([ref[first + j, pl.ds(0, ref.shape[1] - PAD), :] for j in range(n)], 0)

        def put(ref, row, v):
            ref[row // L, pl.ds(row % L // 2, 8), :] = packed(v)

        def channel_rows(j, r0, n):
            par_s[j, pl.ds(r0, n), :] = jnp.broadcast_to(pt_s[pl.ds(r0, n), j:j + 1], (n, L))

        def region(plan, c):
            z = z_s[0]
            zv = jnp.full((8, L), z, jnp.int32).astype(u32)
            prog = Program(c["LEAD"], c["USE"], (c["UN"], (c["PO"], c["PR"]), (c["TO"], c["TR"]), c["EN"], c["GE"], c["PL"], c["PU"], c["PE"]))

            def after(x, todo, tiles=1):
                toks = {}
                for s, fn in todo:
                    for t in fn():
                        toks[s] = toks.get(s, zv) & pltpu.bitcast(t, u32)
                if toks:
                    parts = [x[r:r + 8] for r in range(0, x.shape[0], 8)]
                    for s, t in toks.items():
                        for e in range(tiles):
                            j = (8 * e + s) * (1 if x.dtype == u32 else 2)
                            parts[j] = pltpu.bitcast(pltpu.bitcast(parts[j], u32) | t, x.dtype)
                    x = cat(parts, 0)
                return pltpu.bitcast(x, bf16) if x.dtype == u32 else x.astype(bf16)

            def span(i, a, n):
                return pl.ds(pl.multiple_of(i * TF + a, L), n)

            def colsum(x):
                return jnp.broadcast_to(jnp.sum(x, axis=0, keepdims=True), x.shape)

            def identity(n):
                eye = lax.broadcasted_iota(jnp.int32, (n, n), 0) == lax.broadcasted_iota(jnp.int32, (n, n), 1)
                return eye.astype(f32).astype(bf16)

            def transpose_weight(w_v, base):
                low = lax.broadcasted_iota(jnp.int32, (8, L), 1) < 64
                for c in range(0, D, L):
                    def step(due, c=c):
                        n = min(L, D - c)
                        out = [dot_nt(identity(n), w_v[pl.ds(a, L), pl.ds(c, n)]) for a in (0, L, 2 * L, 384, 448)]
                        for r in range(0, n, 16):
                            t = [packed(y[r:r + 16]) for y in out]
                            t.append(jnp.where(low, t[3], t[4]))
                            for j in range(6):
                                wt_s[base + j, pl.ds((c + r) // 2, 8), :] = t[j]
                        return out
                    prog.step([(min(L, D - c) // 16, 1, 1)] * 5, step, False)
                    yield

            def ln1_tasks(m):
                tl = pl.ds(256 * m, 256)
                ld = lambda r: q_v[0, pl.ds(r, 8), tl].astype(f32)
                tasks = []

                def gated(gt):
                    if gt is not None:
                        q_v[z + 1, pl.ds(0, 8), pl.ds(0, 256)] = cat([gt, gt], 1).astype(bf16)

                for r0 in range(0, D, LR):
                    def sums(gt, r0=r0):
                        gated(gt)
                        xs = [ld(r) for r in range(r0, r0 + LR, 8)]
                        ws = [par_s[5, pl.ds(r, 8), :] for r in range(r0, r0 + LR, 8)]
                        s, g = tree_sum(xs), tree_sum([x * cat([w, w], 1) for x, w in zip(xs, ws)])
                        if r0:
                            s, g = s + st_s[z + 0], g + st_s[z + 1]
                        if r0 + LR < D:
                            st_s[0], st_s[1] = s, g
                        else:
                            st_s[2] = colsum(s) * (1.0 / D)
                            g = jax.nn.sigmoid(colsum(g))
                            g_s[0, :, tl], g_s[1, :, tl] = g, (1.0 - g) * (0.5 / GS)
                        return [st_s[z, :, pl.ds(0, L)]]
                    tasks.append((LR + 4, sums))
                for r0 in range(0, D, LR):
                    def squares(gt, r0=r0):
                        gated(gt)
                        mean = st_s[z + 2]
                        xs = [ld(r) - mean for r in range(r0, r0 + LR, 8)]
                        s = tree_sum([x * x for x in xs])
                        if r0:
                            s = s + st_s[z + 0]
                        if r0 + LR < D:
                            st_s[0] = s
                        else:
                            st_s[3] = lax.rsqrt(colsum(s) * (1.0 / D) + EPS) * GS
                        return [st_s[z, :, pl.ds(0, L)]]
                    tasks.append((LR + 2, squares))
                for r0 in range(0, D, LR):
                    def scale(gt, r0=r0):
                        gated(gt)
                        mean, rstd = st_s[z + 2], st_s[z + 3]
                        for r in range(r0, r0 + LR, 16):
                            x = cat([(ld(r + h) - mean) * rstd for h in (0, 8)], 0)
                            for t, row, v in pair_rows(r, x[:, :L], x[:, L:]):
                                put(xn_s[m % 2], row, v)
                        return [xn_s[m % 2][z, pl.ds(0, 8), :]]
                    tasks.append((LR + 55, scale))
                return tasks

            def pair_rows(r, a, b):
                if r < 384:
                    return [(0, r, a), (1, 512 + r, b)]
                if r < 448:
                    return [(2, 1024 + r - 384, a), (1, 512 + r, b - a)]
                if r < 512:
                    return [(2, 1024 + r - 384, b), (0, r - 64, a - b)]
                return [(0, r - 64, a), (1, 512 + r - 64, b)]

            def pair_steps(m, base, operand, consume):
                for j in range(4):
                    def shared(due, j=j):
                        y = dot(pltpu.bitcast(wt_s[base + 3, pl.ds(72 * j, 72), :], bf16),
                                after(operand(1024, L), due[0]))
                        r_s[m % 2, pl.ds(144 * j, 144), :] = y
                        return [y]
                    prog.step([(9, 1, 0)], shared)
                last = [None]
                for t in range(2):
                    for j in range(4):
                        def own(due, t=t, j=j):
                            w = cat([pltpu.bitcast(wt_s[base + e, pl.ds(72 * j, 72), :], bf16)
                                     for e in (0, 1, 2, 4 + t)], 1)
                            y = dot(w, after(operand(512 * t, 512), due[0], 4))
                            if last[0] is not None:
                                r_s[z + 2, pl.ds(0, 8), :] = last[0]
                            consume(2 * m + t, j, y + r_s[m % 2, pl.ds(144 * j, 144), :], last[0])
                            last[0] = y[RG:RG + 8]
                            return [y]
                        prog.step([(9, 4, 0)], own)

            def put_h(t, j, y, gt):
                h = gelu2(y) * (0.5 / GS)
                h_s[t, pl.ds(144 * j, 144), :] = pltpu.roll(h, SHIFTS[j] % L, axis=1)

            def shift_tasks(m):
                tasks = []
                lane = lax.broadcasted_iota(jnp.int32, (16, L), 1)
                for j, sh in enumerate(SHIFTS):
                    def task(gt, j=j, sh=sh):
                        if gt is not None:
                            h_s[z + NC, pl.ds(0, 8), :] = gt
                        for r in range(144 * j, 144 * j + 144, 16):
                            rot = lambda t: h_s[t, pl.ds(r, 16), :]
                            a, b = rot(2 * m), rot(2 * m + 1)
                            if sh > 0:
                                c = rot(2 * m - 1) if m else jnp.zeros_like(a)
                                a, b = jnp.where(lane >= sh, a, c), jnp.where(lane >= sh, b, a)
                            else:
                                c = rot(2 * m + 2) if 2 * m + 2 < NC else jnp.zeros_like(a)
                                a, b = jnp.where(lane < L + sh, a, b), jnp.where(lane < L + sh, b, c)
                            for t, row, v in pair_rows(r, a, b):
                                put(hs_s[m % 2], row, v)
                        return [hs_s[m % 2][z, pl.ds(0, 8), :]]
                    tasks.append((130, task))
                return tasks

            total = {}

            def put_x1(t, j, y, gt):
                tl, rows = pl.ds(t * L, L), pl.ds(144 * j, 144)
                if gt is not None:
                    q_v[z + 1, pl.ds(0, 8), pl.ds(0, 256)] = cat([gt, gt], 1).astype(bf16)
                x1 = y + q_v[0, rows, tl].astype(f32)
                ga_s[rows, tl] = x1 * cat([1.0 - g_s[0, :, tl]] * 18, 0)
                x1_s[t // 2][t % 2, rows, :] = x1
                s = x1[0:8] + total[t] if j else x1[0:8]
                for r in range(8, 144, 8):
                    s = s + x1[r:r + 8]
                total[t] = s
                if j == 3:
                    x1_s[t // 2][2, pl.ds(8 * (t % 2), 8), :] = colsum(s) * (1.0 / D)

            def ln2_tasks(m):
                tasks = []
                for t in (2 * m, 2 * m + 1):
                    for r0 in range(0, D, 144):
                        def squares(gt, t=t, r0=r0):
                            if gt is not None:
                                x1_s[m][z + 2, pl.ds(32, 8), :] = gt
                            mean = x1_s[m][2, pl.ds(8 * (t % 2), 8), :]
                            xs = [x1_s[m][t % 2, pl.ds(r, 8), :] - mean for r in range(r0, r0 + 144, 8)]
                            s = tree_sum([x * x for x in xs])
                            if r0:
                                s = s + st_s[z + 4, :, pl.ds(0, L)]
                            if r0 + 144 < D:
                                st_s[4, :, pl.ds(0, L)] = s
                            else:
                                s = lax.rsqrt(colsum(s) * (1.0 / D) + EPS) * GS
                                x1_s[m][2, pl.ds(16 + 8 * (t % 2), 8), :] = s
                            return [s]
                        tasks.append((18 * 3 + 2, squares))
                return tasks

            def scale_tasks(m):
                tasks = []
                for t in range(2):
                    for e, parts in enumerate((((0, L),), ((L, 64), (L, 64)), ((192, L),), ((320, L),), ((448, L),))):
                        def task(gt, t=t, e=e, parts=parts):
                            if gt is not None:
                                x1_s[m][z + 2, pl.ds(32, 8), :] = gt
                            mean, rstd = (x1_s[m][2, pl.ds(o + 8 * t, 8), :] for o in (0, 16))
                            xq_s[m % 2][5 * t + e, pl.ds(0, L), :] = cat([
                                (x1_s[m][t, pl.ds(a + r, 8), :] - mean) * rstd for a, n in parts for r in range(0, n, 8)], 0)
                            return [xq_s[m % 2][z, pl.ds(0, 8), :]]
                        tasks.append((34, task))
                return tasks

            def turn(m):
                for t in range(2):
                    def step(due, t=t):
                        y = dot_nt(identity(L), after(stacked(xq_s[m % 2], 5 * t, 5), due[0]))
                        for e in range(5):
                            xp_s[m // 4][4 * e + m % 4, pl.ds(L * t, L), :] = y[:, L * e:L * e + L]
                        return [y]
                    prog.step([(8, 5, 1)], step)

            def xa_tasks(sb):
                tasks = []
                low = lax.broadcasted_iota(jnp.int32, (16, L), 1) < 64
                for p1 in range(7):
                    for s in range(8):
                        def task(gt, p1=p1, s=s):
                            if gt is not None:
                                xp_s[sb][z + 20, pl.ds(0, 8), :] = gt
                            x, y = [], []
                            for g in range(2):
                                ld = lambda e, t1, t2: xp_s[sb][4 * e + 2 * t1 + t2, pl.ds(L * g + 16 * s, 16), :]
                                l1 = {(t2, k2): lin(A_TERMS[p1], lambda t1, k1: ld((0, 2, 3, 4)[2 * k1 + k2], t1, t2))
                                      for t2, k2 in QUADS}
                                x.append([lin(A_TERMS[p2], lambda t2, k2: l1[t2, k2]) for p2 in range(7)])
                                if p1 in LONG:
                                    e1 = [lin(A_TERMS[p1], lambda t1, k1: None if k1 else ld(1, t1, t2)) for t2 in range(2)]
                                    y.append({p2: lin(A_TERMS[p2], lambda t2, k2: None if k2 else e1[t2]) for p2 in LONG})
                            v = []
                            for p2 in range(7):
                                a, b = x[0][p2], x[1][p2]
                                if long_[p1 * 7 + p2]:
                                    v += [jnp.where(low, a, b), jnp.where(low, y[0][p2], a - b),
                                          jnp.where(low, b - a, y[1][p2])]
                                else:
                                    v += [a, b]
                            for c, u in enumerate(v):
                                xa_s[sb][cols[7 * p1] + c, pl.ds(8 * s, 8), :] = packed(u)
                            return [xa_s[sb][z, pl.ds(0, 8), :]]
                        tasks.append(((24 if p1 in LONG else 16) * len(A_TERMS[p1]) + (138 if p1 in LONG else 74), task))
                return tasks

            def b_tasks(i):
                tasks = []
                for s in range(12):
                    for group in (((0, 1), (4,), (2, 5), (3, 6)) if s < 8 else (LONG,)):
                        def task(gt, group=group, s=s):
                            if gt is not None:
                                w3_v[pl.ds(0, 8), span(z + NF, 0, 256)] = cat([gt, gt], 1).astype(bf16)

                            def block(k1, f1, k2):
                                if s >= 8 and (k1 or k2):
                                    return None
                                rows = pl.ds(QUARTER[2 * k1 + k2] + 16 * s, 16)
                                return w3_v[rows, span(i, 256 * f1, 256)].astype(f32)
                            for p1 in group:
                                l1 = [lin(B_TERMS[p1], lambda k1, f1: block(k1, f1, k2)) for k2 in range(2)]
                                for p2 in (range(7) if s < 8 else LONG):
                                    v = lin(B_TERMS[p2],
                                            lambda k2, f2: None if l1[k2] is None else l1[k2][:, L * f2:L * f2 + L])
                                    if len(B_TERMS[p1]) == len(B_TERMS[p2]) == 1:
                                        (_, k1, f1), (_, k2, f2) = B_TERMS[p1][0], B_TERMS[p2][0]
                                        v = pltpu.bitcast(w3_v[pl.ds(QUARTER[2 * k1 + k2] + 16 * s, 16),
                                                               span(i, 256 * f1 + L * f2, L)], u32)
                                    b_s[p1 * 7 + p2, pl.ds(8 * s, 8), :] = v if v.dtype == u32 else packed(v)
                            return [b_s[z, pl.ds(0, 8), :]]
                        tasks.append((55 * len(group) if s < 8 else 60, task))
                return tasks

            def a_tasks(i):
                tasks = []
                for s in range(18):
                    for f in range(2):
                        def task(gt, s=s, f=f):
                            if gt is not None:
                                w4_v[pl.ds(0, 8), span(z + NF, 0, 256)] = cat([gt, gt], 1).astype(bf16)
                            xs = {(r, c): w4_v[pl.ds(288 * r + 16 * s, 16), span(i, 256 * c, 256)].astype(f32)
                                  for r, c in QUADS}
                            for p, terms in enumerate(A_TERMS):
                                v = lin(terms, lambda r, c: xs[r, c][:, L * f:L * f + L])
                                if len(terms) == 1:
                                    _, r, c = terms[0]
                                    v = pltpu.bitcast(w4_v[pl.ds(288 * r + 16 * s, 16), span(i, 256 * c + L * f, L)], u32)
                                a_s[2 * p + f, pl.ds(8 * s, 8), :] = v if len(terms) == 1 else packed(v)
                            return [a_s[z, pl.ds(0, 8), :]]
                        tasks.append((55, task))
                return tasks

            def first_matmul(sb):
                for p in range(49):
                    def step(due, p=p):
                        xa = lambda c: pltpu.bitcast(xa_s[sb][cols[p] + c, pl.ds(0, 64), :], bf16)
                        bt = lambda a, m: b_s[p, pl.ds(a // 2, m // 2), :]
                        if long_[p]:
                            tiles = [bt(0, L), cat([bt(L, 64), bt(64, 64)], 0), cat([bt(0, 64), bt(L, 64)], 0)]
                            r, a, b = out = [dot(xa(j), after(tiles[j], due[j])) for j in range(3)]
                            a, b = a + r, b + r
                        else:
                            out = [dot(cat([xa(0), xa(1)], 0), after(bt(0, L), due[0]))]
                            a, b = out[0][:L], out[0][L:]
                        for g, y in enumerate((a, b)):
                            p_s[sb][p, pl.ds((L + PAD) * g, L), :] = y
                        return out
                    prog.step([(8, 1, 0)] * 3 if long_[p] else [(16, 1, 0)], step)
                    yield

            def second_matmul(sb, by_tokens=False):
                n = 18 // RS
                parts = [(p, t, n * h, n) for p in range(7) for t in range(4) for h in range(RS)]
                parts = [(0, 0, 0, n // 2)] + parts[1:] + [(0, 0, n // 2, n - n // 2)]
                if by_tokens:
                    parts.sort(key=lambda e: e[1] // 2)
                for e, (p, t, r0, n) in enumerate(parts):
                    def step(due, e=e, p=p, t=t, r0=r0, n=n):
                        a = cat([pltpu.bitcast(a_s[2 * p + f, pl.ds(8 * r0, 8 * n), :], bf16) for f in range(2)], 1)
                        g = cat([u_s[sb][7 * (2 * (t // 2) + f) + p, pl.ds(64 * (t % 2), 64), :] for f in range(2)], 0)
                        g = after(g, due[0], 2)
                        y = dot_nt(a, cat([g[:L], g[L:]], 1))
                        acc_s[2 * sb + t // 2][7 * (t % 2) + p, pl.ds(16 * r0, 16 * n), :] += y
                        return [y]
                    prog.step([(n, 2, 1)], step)
                    for _ in range((e + 1) * 50 // len(parts) - e * 50 // len(parts)):
                        yield

            def gelu_tasks(sb, first, last):
                tasks = []
                for j in range(first, last):
                    for q in ((0, 0), (1, 1), (0, 1), (1, 0)):
                        def task(gt, g=j % 2, r=16 * (j // 2), q=q):
                            if gt is not None:
                                p_s[sb][z + 49, pl.ds(0, 8), :] = gt
                            rows = pl.ds((L + PAD) * g + r, 16)
                            m = [combine(lambda p2: p_s[sb][7 * p1 + p2, rows, :], q) for p1 in range(7)]
                            h = {ij: gelu2(combine(lambda p1: m[p1], ij)) for ij in QUADS}
                            for p in range(7):
                                v = lin(B_TERMS[p], lambda r1, c1: h[c1, r1])
                                u_s[sb][7 * QUADS.index(q) + p, pl.ds(64 * g + r // 2, 8), :] = packed(v)
                            return [u_s[sb][z, pl.ds(0, 8), :]]
                        tasks.append((145 if q[0] == q[1] else 117, task))
                return tasks

            def out_tasks(sb, halves):
                tasks = []
                for r in range(0, 288, 8):
                    for t2 in halves:
                        def task(gt, r=r, t2=t2):
                            if gt is not None:
                                acc_s[2 * sb + t2][z + 14, pl.ds(0, 8), :] = gt
                            m = [cat([acc_s[2 * sb + t2][7 * j + p, pl.ds(r, 8), :] for j in range(2)], 1) for p in range(7)]
                            for d1, t1 in QUADS:
                                rows, tl = pl.ds(288 * d1 + r, 8), pl.ds(1024 * sb + 512 * t1 + 256 * t2, 256)
                                y = combine(lambda p: m[p], (d1, t1))
                                o_v[rows, tl] = (ga_s[rows, tl] + g_s[1, :, tl] * y).astype(bf16)
                            return [y[:, :L]]
                        tasks.append((38, task))
                return tasks

            def chans(i, r):
                return pl.ds(pl.multiple_of(i * CG + 16 * r, 16), 16)

            def dft(due):
                f = after(stacked(f_s, 0, 2), due)
                return cat([f[:L], f[L:]], 1)

            def kernel_spectrum(i, r):
                def step(due):
                    y = dot(cat([kk_v[chans(i, r), pl.ds(c * L, L)] for c in range(NC)], 0),
                            dft(due[0]))
                    for c in range(NC):
                        a, b = y[16 * c:16 * c + 16, :L], y[16 * c:16 * c + 16, L:]
                        if c == 0:
                            a = a + par_s[4, chans(i, r), :]
                            re, im = a, b
                        else:
                            re, im = a + pb, b - pa
                        pa, pb = a, b
                        rows = pl.ds(16 * c, 16)
                        c_s[r][3, rows, :] = re
                        c_s[r][4, rows, :] = im - re
                        c_s[r][5, rows, :] = re + im
                    return [y]
                prog.step([(16, 2, 0)], step)

            def kv_tasks(i, r):
                tasks = []
                lane = lax.broadcasted_iota(jnp.int32, (16, L), 1)
                for c0 in range(0, NC, KG):
                    def task(gt, c0=c0):
                        if gt is not None:
                            kv_v[z + 1, pl.ds(D, 8), pl.ds(0, 256)] = cat([gt, gt], 1).astype(bf16)
                        ld = lambda o, c: kv_v[o, chans(i, r), pl.ds(c * L, L)].astype(f32)
                        tap = [par_s[j, chans(i, r), :] for j in range(4)]
                        prev = [pltpu.roll(ld(0, c0 - 1), j, axis=1) for j in range(1, 4)] if c0 else None
                        for c in range(c0, c0 + KG):
                            k = ld(0, c)
                            rot = [pltpu.roll(k, j, axis=1) for j in range(1, 4)]
                            ks = k * tap[0]
                            for j in range(1, 4):
                                ks = ks + jnp.where(lane >= j, rot[j - 1], prev[j - 1] if prev else 0.0) * tap[j]
                            prev = rot
                            kvp_s[r][0, pl.ds(16 * c, 16), :] = (ks * ld(1, c)).astype(bf16)
                        return [kvp_s[r][z, pl.ds(0, 16), :]]
                    tasks.append((28 * KG, task, c["XE"] // 2))
                return tasks

            def signal_spectrum(i, r):
                def step(due):
                    y = dot(kvp_s[r][0], dft(due[0]))
                    for j, v in enumerate((y[:, :L], y[:, L:], y[:, :L] + y[:, L:])):
                        c_s[r][j, pl.ds(0, 16 * NC), :] = v
                    return [y]
                prog.step([(16, 2, 0)], step)

            def product_tasks(r):
                tasks = []
                for c0 in range(0, NC, CB):
                    held = {}

                    def task(gt, hf, c0=c0, held=held):
                        if gt is not None:
                            c_s[r][z + 6, pl.ds(0, 8), :] = gt
                        cache = {}

                        def ld(j, c):
                            if (j, c) not in cache:
                                cache[j, c] = c_s[r][j, pl.ds(16 * c + 8 * hf, 8), :]
                            return cache[j, c]
                        acc = {}
                        for j in range(c0 + CB):
                            for c in range(max(j, c0), c0 + CB):
                                t = (ld(3, j) * ld(2, c - j), ld(4, j) * ld(0, c - j), ld(5, j) * ld(1, c - j))
                                acc[c] = t if j == 0 else tuple(a + b for a, b in zip(acc[c], t))
                        for c in range(c0, c0 + CB):
                            held[hf, c] = (acc[c][0] - acc[c][2], acc[c][0] + acc[c][1])
                            if hf:
                                for e in range(2):
                                    y_s[r][e, pl.ds(16 * c, 16), :] = cat([held[0, c][e], held[1, c][e]], 0).astype(bf16)
                        if hf:
                            return [y_s[r][z, pl.ds(0, 16), :]]
                        return [v for c in range(c0, c0 + CB) for v in held[0, c]]
                    cost = sum(6 * (c + 1) + 1 for c in range(c0, c0 + CB)) + 2
                    tasks += [(cost, lambda gt, hf=hf, f=task: f(gt, hf)) for hf in range(2)]
                return tasks

            def inverse(i, r):
                def step(due):
                    y = dot_nt(cat([y_s[r][j, pl.ds(0, 16 * NC), :] for j in range(2)], 1), dft(due[0]))
                    for c in range(NC):
                        tl = pl.ds(c * L, L)
                        g = g_s[0, :, tl] * (1.0 / L)
                        ga_s[chans(i, r), tl] += y[16 * c:16 * c + 16] * (q_v[0, chans(i, r), tl].astype(f32) * cat([g, g], 0))
                    return [y]
                prog.step([(16, 2, 1)], step)

            plan(prog, dict(
                ln1=ln1_tasks, pair=pair_steps, put_h=put_h, shift=shift_tasks, put_x1=put_x1, ln2=ln2_tasks, wt=transpose_weight, scale=scale_tasks, turn=turn,
                xa=xa_tasks, b=b_tasks, a=a_tasks, d1=first_matmul, d2=second_matmul, gelu=gelu_tasks, out=out_tasks,
                ks=kernel_spectrum, kv=kv_tasks, xs=signal_spectrum, prod=product_tasks, inv=inverse))
            prog.emit()

        def run(prog, steps, hooks, times, base=0):
            for p, _ in enumerate(steps):
                for name, fn in hooks.get(base + p, ()):
                    times[name + "<"] = prog.now()
                    fn()
                    times[name], times[name + "#"] = prog.now(), len(prog.steps) - 1
            return prog.now()

        def conv_hooks(w, i, kp, xp, ip):
            hooks = {}
            for r in range(4):
                for name, pos in (("ks", kp), ("xs", xp), ("inv", ip)):
                    hooks.setdefault(pos[r], []).append((name + str(r), lambda name=name, r=r: w[name](i, r)))
            return hooks

        def conv_tasks(prog, w, i, times, t, first, c):
            LE, LX = c["LE"], c["LX"]
            for r in range(4):
                prog.spread(w["kv"](i, r), t, times["xs%d<" % r] - LX, first, times["xs%d#" % r])
                t = times["xs%d<" % r] - LX
            t = 0
            for r in range(4):
                t0 = max(t, times["xs%d" % r] + LE)
                t = times["inv%d<" % r] - LX
                prog.spread(w["prod"](r), t0, t, max(times["xs%d#" % r], times["ks%d#" % r]) + 1, times["inv%d#" % r])

        def head(prog, w):
            LE, LX = H["LE"], H["LX"]
            for c in small + [w1_copy, q_first]:
                c.wait()
            for c in q_second + q_rest:
                c.start()
            pt_s[...] = cat([sh_v[...].astype(f32), d_v[...].astype(f32).reshape(1, D),
                             gw_v[...].astype(f32).reshape(1, D), jnp.zeros((2, D), f32)], 0).T
            channel_rows(5, 0, D)
            run(prog, w["wt"](w1_v, 0), {}, {})

            def first_pair(due):
                done = [None] * 2
                for _, fn in w["ln1"](0):
                    done += [pltpu.bitcast(x, f32) for x in fn(done[-2])]
            prog.step([], first_pair)
            t, k = [prog.now()], [len(prog.steps)]
            second = w["wt"](w2_v, 6)
            for m in range(8):
                for _ in range(WP.count(m)):
                    next(second)
                w["pair"](m, 0, lambda r, n, m=m: stacked(xn_s[m % 2], r // L, n // L), w["put_h"])
                t.append(prog.now())
                k.append(len(prog.steps))
            turned = []
            for m in range(8):
                w["pair"](m, 6, lambda r, n, m=m: stacked(hs_s[m % 2], r // L, n // L), w["put_x1"])
                if m:
                    turned.append((prog.now(), len(prog.steps)))
                    w["turn"](m - 1)
                t.append(prog.now())
                k.append(len(prog.steps))
            steps = w["d1"](0)
            run(prog, zip(range(T7), steps), {}, {})
            turned.append((prog.now(), len(prog.steps)))
            w["turn"](7)
            t7, k7 = prog.now(), len(prog.steps)
            run(prog, zip(range(49 - T7 - TE), steps), {}, {})
            t1 = prog.now()
            run(prog, steps, {}, {})

            def exchange(waits, starts):
                def fn(gt):
                    for c in waits:
                        c.wait()
                    for c in starts:
                        c.start()
                    return []
                return [(1, fn)]

            def clear(gt, sb, j):
                acc_s[sb][j, pl.ds(0, 288), :] = jnp.zeros((288, L), f32)
                return [acc_s[sb][z_s[0], pl.ds(0, 8), :]]

            def rows(gt, j, r0):
                channel_rows(j, r0, CG)
                return []

            prog.spread(merge([(1, lambda gt, sb=sb, j=j: clear(gt, sb, j)) for sb in range(len(acc_s)) for j in range(acc_s[0].shape[0] - 1)],
                              [(1, lambda gt, j=j, r=r: rows(gt, j, r)) for r in range(0, D, CG) for j in range(5)]),
                        t[0], t[8], k[0], k[8])
            for m in range(1, 8):
                pre = {2: exchange(q_second, early), 4: exchange(q_rest, [])}.get(m, [])
                prog.spread(pre + w["ln1"](m), t[m - 1], t[m] - L1, k[m - 1], k[m])
            prog.spread(exchange(early, then + late), t[XW], t[XW] + 20, k[XW], k[XW] + 6)
            prog.spread(w["shift"](0), t[6], t[8] - 36, k[6], k[8])
            for m in range(1, 8):
                prog.spread(w["shift"](m), t[7 + m] + LE, t[8 + m] - 36, k[7 + m], k[8 + m])
            for m in range(8):
                prog.spread(w["ln2"](m) + w["scale"](m), t[9 + m] + LE * (m == 0), turned[m][0] - LX, k[9 + m], turned[m][1])
            prog.spread(w["b"](0), t[8], t[13], k[8], k[13])
            prog.spread(w["xa"](0), t[13] + LE, t[16] - XL, k[13], k[16])
            prog.spread(w["xa"](1), t7 + LE, t1, k7, len(prog.steps))

            def first_half(due):
                done = [None] * 2
                for _, fn in w["gelu"](0, 0, EA):
                    done += [pltpu.bitcast(x, f32) for x in fn(done[-2])]
            prog.step([], first_half)

        def middle(i):
            def plan(prog, w):
                LE, LX = M["LE"], M["LX"]
                times = {}
                hooks = conv_hooks(w, i, KP, XP, IP)
                t1 = run(prog, w["d1"](1), hooks, times, 0)
                k1 = len(prog.steps)
                t2 = run(prog, w["d2"](0), hooks, times, 49)
                k2 = len(prog.steps)
                t3 = run(prog, w["d1"](0), hooks, times, 99)
                k3 = len(prog.steps)
                t4 = run(prog, w["d2"](1), hooks, times, 148)
                prog.spread(merge(w["a"](i), w["gelu"](0, EA, 16)), 0, t1 - LX, 0, k1)
                prog.spread(merge(w["b"](i + 1), w["gelu"](1, 0, EB)), t1 + LE, t2 - LX, k1, k2)
                prog.spread(w["gelu"](1, EB, 16), t2 - LX, t3 - LX, k2, k3)
                prog.spread(w["gelu"](0, 0, EA), t3 + LE, t4, k3, len(prog.steps))
                conv_tasks(prog, w, i, times, times["xs0<"] - KW, 0, M)

            @pl.when(i == 1)
            def _():
                for c in late:
                    c.wait()
            region(plan, M)

        def tail(prog, w):
            LE, LX = T["LE"], T["LX"]
            times = {}
            hooks = conv_hooks(w, NF - 1, CK, CX, CI)
            t1 = run(prog, w["d1"](1), hooks, times)
            k1 = len(prog.steps)
            t2 = run(prog, w["d2"](0), hooks, times, 49)
            run(prog, [0], hooks, times, 99)
            conv_tasks(prog, w, NF - 1, times, 0, 0, T)
            k2 = len(prog.steps)
            steps = w["d2"](1, True)
            t3 = run(prog, zip(range(25), steps), {}, {})
            k3 = len(prog.steps)
            t4 = run(prog, steps, {}, {})
            assert k3 - k2 == 14 * RS + 1
            prog.spread(merge(w["a"](NF - 1), w["gelu"](0, EA, 16)), 0, t1 - LX, 0, k1)
            prog.spread(w["gelu"](1, 0, 16), t1 + LE, t2 - LX, k1, k2)

            def send(copies):
                return [(1, lambda gt: [c.start() for c in copies] * 0)]
            prog.spread(w["out"](0, (0, 1)) + send(out[0]), t2 + LE, t2 + (t3 - t2) * TS0, k2, k3)
            prog.spread(w["out"](1, (0,)) + send(out[1]), t3 + LE, t3 + (t4 - t3) * TS, k3, len(prog.steps))

            def finish(due):
                done = [None] * FL
                for _, fn in w["out"](1, (1,)):
                    done += fn(done[-FL])
                for c in out[2]:
                    c.start()
            prog.step([], finish)

        region(head, H)
        for c in then:
            c.wait()
        pl.loop(0, NF - 1)(middle)
        region(tail, T)
        for c in sum(out, []):
            c.wait()

    V = pltpu.VMEM
    scratch = [
        V((2, D, S + L), bf16), V((2, D + 16, S + L), bf16), V((D, S + L), bf16),
        V((D, D), bf16), V((D, D), bf16), V((D, F + 256), bf16), V((D, F + 256), bf16),
        V((4, D), bf16), V((D,), bf16), V((D,), bf16), V((D, S + L), bf16),
        V((D, 8), f32), V((6, D + PAD, L), f32), V((2, 64 + PAD, L), u32), V((12, D // 2 + PAD, L), u32),
        V((6, 8, 2 * L), f32), V((3, D + PAD, L), f32), [V((9, 64 + PAD, L), u32)] * 2, V((NC + 1, D + PAD, L), f32),
        [V((9, 64 + PAD, L), u32)] * 2, [V((3, D + PAD, L), f32)] * 8, [V((10, L + PAD, L), f32)] * 2, [V((21, 256 + PAD, L), f32)] * 2, [V((nxt, 64 + PAD, L), u32)] * 2,
        V((2, 8, S), f32), V((D, S + L), f32),
        [V((15, 288 + PAD, L), f32)] * 4, [V((50, 256 + 3 * PAD, L), f32)] * 2, [V((28, L + PAD, L), u32)] * 2,
        V((49, 96 + PAD, L), u32), V((14, 144 + PAD, L), u32),
        [V((7, 16 * NC + PAD, L), f32)] * 4, [V((1, 16 * NC, L), bf16)] * 4, [V((2, 16 * NC + 2 * PAD, L), bf16)] * 4,
        pltpu.SMEM((2,), jnp.int32),
        pltpu.SemaphoreType.DMA((29,)),
    ]

    def fn(A_q, A_k, A_v, A_shift_k, A_ssm_k, A_ssm_D, B_x, B_w1, B_w2, B_w3, B_w4, gate_w):
        del B_x
        t = lambda a: jnp.swapaxes(a[0], 0, 1)
        hbm = pl.BlockSpec(memory_space=pl.ANY)
        out = pl.pallas_call(
            kern, out_shape=spec((D, S), bf16), in_specs=[hbm] * 11, out_specs=hbm, scratch_shapes=scratch,
            compiler_params=pltpu.CompilerParams(vmem_limit_bytes=120 * 1024 * 1024),
        )(t(A_q), t(A_k), t(A_v), A_shift_k.T, A_ssm_k, A_ssm_D, B_w1, B_w2, B_w3, B_w4.T, gate_w)
        return jnp.swapaxes(out, 0, 1)[None]

    return fn


@jax.jit
def pallas_gated_mix__ssm_conv_h3__mixer_s_mlp__prompt_kernel(
    A_q, A_k, A_v, A_shift_k, A_ssm_k, A_ssm_D, B_x, B_w1, B_w2, B_w3, B_w4, gate_w
):
    fn = build()
    return fn(A_q, A_k, A_v, A_shift_k, A_ssm_k, A_ssm_D, B_x, B_w1, B_w2, B_w3, B_w4, gate_w)
```
